```python
import os as _os
_os.environ.setdefault("JAX_PLATFORMS", "cpu")
import jax
import jax.numpy as jnp

def _softmax(x, axis=-1):
    return jax.nn.softmax(x, axis=axis)
def _gelu(x):
    return jax.nn.gelu(x, approximate=True)
def _silu(x):
    return jax.nn.silu(x)
def _sigmoid(x):
    return jax.nn.sigmoid(x)
def _layernorm(x, axis=-1, eps=1e-5):
    m = jnp.mean(x, axis=axis, keepdims=True)
    v = jnp.var(x, axis=axis, keepdims=True)
    return (x - m) / jnp.sqrt(v + eps)
def _scatter_add(tgt, idx, src, axis=0):
    return tgt.at[idx].add(src)
def _segment_sum(src, seg, n):
    return jax.ops.segment_sum(src, seg, n)
class _Rng:
    def __init__(self, key):
        self._k = key
    def _next(self):
        self._k, sub = jax.random.split(self._k)
        return sub
    def normal(self, shape):
        return jax.random.normal(self._next(), shape, dtype=jnp.bfloat16)
    def randint(self, lo, hi, shape):
        return jax.random.randint(self._next(), shape, lo, hi, dtype=jnp.int32)
    def uniform(self, shape, lo=0.0, hi=1.0):
        return jax.random.uniform(self._next(), shape, jnp.bfloat16, lo, hi)
    def permutation(self, n):
        return jax.random.permutation(self._next(), n)


kernel_name = 'gated_mix__mha_block__mha_block__prompt'

def setup_inputs():
    _rng = _Rng(jax.random.key(int.from_bytes(__import__("os").urandom(4), "little")))
    _w = (lambda a: (lambda t: t.astype(jnp.bfloat16) if jnp.issubdtype(t.dtype, jnp.floating) else t)(jnp.asarray(a)))
    def _A_setup():
        B, S, D, H = 1, 2048, 448, 16
        return {
            "x": _w((lambda *s: _rng.normal(s) * 0.05)(B, S, D)),
            "wqkv": _w((lambda *s: _rng.normal(s) * 0.4)(D, 3 * D)),
            "wo": _w((lambda *s: _rng.normal(s) * 0.05)(D, D)),
        }
    _A_in = _A_setup()

    def _B_setup():
        B, S, D, H = 1, 2048, 448, 16
        return {
            "x": _w((lambda *s: _rng.normal(s) * 0.05)(B, S, D)),
            "wqkv": _w((lambda *s: _rng.normal(s) * 0.4)(D, 3 * D)),
            "wo": _w((lambda *s: _rng.normal(s) * 0.05)(D, D)),
        }
    _B_in = _B_setup()

    return {
        "A_x": _A_in["x"],
        "A_wqkv": _A_in["wqkv"],
        "A_wo": _A_in["wo"],
        "B_x": _B_in["x"],
        "B_wqkv": _B_in["wqkv"],
        "B_wo": _B_in["wo"],
        "gate_w": _w((lambda *s: _rng.normal(s) * 0.05)(448) * 16.0),
    }

def reference(A_x, A_wqkv, A_wo, B_x, B_wqkv, B_wo, gate_w):
    def _A_ref(x, wqkv, wo):
        B, S, D = x.shape
        H = 16
        Dh = D // H
        qkv = (lambda x, *d: x.transpose(*d))((x @ wqkv).reshape(B, S, 3, H, Dh), 2, 0, 3, 1, 4)
        q, k, v = qkv[0], qkv[1], qkv[2]
        scores = jnp.einsum("bhqd,bhkd->bhqk", q, k) * (Dh ** -0.5)
        p = _softmax(scores, axis=-1)
        o = jnp.einsum("bhqk,bhkd->bhqd", p, v)
        return (lambda x, *d: x.transpose(*d))(o, 0, 2, 1, 3).reshape(B, S, D) @ wo

    def _B_ref(x, wqkv, wo):
        B, S, D = x.shape
        H = 16
        Dh = D // H
        qkv = (lambda x, *d: x.transpose(*d))((x @ wqkv).reshape(B, S, 3, H, Dh), 2, 0, 3, 1, 4)
        q, k, v = qkv[0], qkv[1], qkv[2]
        scores = jnp.einsum("bhqd,bhkd->bhqk", q, k) * (Dh ** -0.5)
        p = _softmax(scores, axis=-1)
        o = jnp.einsum("bhqk,bhkd->bhqd", p, v)
        return (lambda x, *d: x.transpose(*d))(o, 0, 2, 1, 3).reshape(B, S, D) @ wo

    x = A_x
    g = _sigmoid((x * gate_w).sum(-1, keepdims=True))
    a = _A_ref(x, A_wqkv, A_wo)
    b = _B_ref(x, B_wqkv, B_wo)
    return g * a + (1 - g) * b
```

```python
import jax
import jax.numpy as jnp
from jax.experimental import pallas as pl
from jax.experimental.pallas import tpu as pltpu

S, D, H, DH, DP = 2048, 448, 16, 28, 32
G = 4 * DH
NQ = 1024
KB = 1024
PT = 512
LOG2E = 1.4426950408889634
QSCALE = DH ** -0.5 * LOG2E
F32, BF16 = jnp.float32, jnp.bfloat16
HI, LO = 2.0 ** 120, 2.0 ** -60
WR = 2 * D + H * DP


def _tr(a):
    a = jnp.concatenate([a.astype(F32), jnp.zeros((512 - D, a.shape[1]), F32)], axis=0)
    return a.T[:, :D]


def _kernel(xt_ref, wqa, woa, wqb, wob, gw, o_ref, q_s, k_s, vt_s, ot_s, w_s, wo_s, g_s):
    i = pl.program_id(0)

    @pl.when(i == 0)
    def _():
        for m, (w_ref, wo_ref) in enumerate(((wqa, woa), (wqb, wob))):
            for c in range(0, 2 * D, 128):
                w_s[c:c + 128, :] = _tr(w_ref[:, c:c + 128]).astype(BF16)
            wv = jnp.concatenate([_tr(w_ref[:, 2 * D + c:2 * D + c + 128]) for c in range(0, 384, 128)]
                                 + [_tr(w_ref[:, 3 * D - 128:3 * D])[64:, :]], axis=0)
            for h in range(H):
                blk = jnp.concatenate([wv[h * DH:(h + 1) * DH, :], jnp.zeros((DP - DH, D), F32)], axis=0)
                w_s[2 * D + h * DP:2 * D + (h + 1) * DP, :] = blk.astype(BF16)
            if m == 0:
                w_s[2 * D + DH + 2:2 * D + DH + 4, :] = jnp.broadcast_to(gw[...].reshape(1, D), (2, D))
            wo = wo_ref[...].astype(F32)
            wop = jnp.concatenate(
                [p for h in range(H) for p in (wo[h * DH:(h + 1) * DH, :], jnp.zeros((DP - DH, D), F32))], axis=0)
            wop = jnp.concatenate([wop, jnp.zeros((H * DP, 512 - D), F32)], axis=1)
            wo_s[:, m * 512:(m + 1) * 512] = wop.T[:D, :].astype(BF16)

            def proj(r, c):
                cols = pl.ds(pl.multiple_of(r * PT, PT), PT)
                t = jnp.dot(w_s[...], xt_ref[:, cols], preferred_element_type=F32)
                for j in range(4):
                    q_s[m * 4 + j, 0:G, cols] = (t[j * G:(j + 1) * G, :] * QSCALE).astype(BF16)
                    lo = D + j * G
                    k_s[cols, (m * 4 + j) * 128:(m * 4 + j + 1) * 128] = t[lo:lo + 128, :].T.astype(BF16)
                v = t[2 * D:, :]
                if m == 0:
                    g_s[:, cols] = jax.nn.sigmoid(v[DH + 2:DH + 3, :])
                ri = jax.lax.broadcasted_iota(jnp.int32, v.shape, 0) % DP
                vt_s[m * 512:(m + 1) * 512, cols] = jnp.where(ri < DH, v, jnp.where(ri == DH, 1.0, 0.0)).astype(BF16)
                return c
            jax.lax.fori_loop(0, S // PT, proj, 0)
        q_s[:, G:, :] = jnp.zeros((8, 128 - G, S), BF16)

    qcols = pl.ds(pl.multiple_of(i * NQ, NQ), NQ)

    def qmasked(h):
        grp = pl.ds(pl.multiple_of((h // 4) * 128, 128), 128)
        qg = q_s[h // 4, :, qcols]
        row = jax.lax.broadcasted_iota(jnp.int32, qg.shape, 0) - (h % 4) * DH
        return grp, jnp.where((row >= 0) & (row < DH), qg, jnp.zeros_like(qg))

    def finish(h, acc):
        hr = pl.ds(pl.multiple_of(h * DP, DP), DP)
        ot_s[hr, :] = (acc * (1.0 / acc[DH:DH + 1, :])).astype(BF16)

    def head(h, bad):
        grp, qm = qmasked(h)
        hr = pl.ds(pl.multiple_of(h * DP, DP), DP)
        acc = jnp.zeros((DP, NQ), F32)
        for kb in range(S // KB):
            ks = slice(kb * KB, (kb + 1) * KB)
            st = jnp.dot(k_s[ks, grp], qm, preferred_element_type=F32)
            p = jnp.exp2(st).astype(BF16)
            acc = acc + jnp.dot(vt_s[hr, ks], p, preferred_element_type=F32)
        finish(h, acc)
        row = jax.lax.broadcasted_iota(jnp.int32, acc.shape, 0)
        ok = (jnp.abs(acc) <= HI) & ((row != DH) | (acc >= LO))
        b = jnp.where(ok, 0.0, 1.0)
        return jnp.maximum(bad, jnp.max(b.reshape(DP // 8, 8, NQ), axis=0))
    bad = jax.lax.fori_loop(0, 2 * H, head, jnp.zeros((8, NQ), F32))

    @pl.when(jnp.max(bad) > 0.0)
    def _():
        SB = 256

        def head_safe(h, c):
            grp, qm = qmasked(h)
            hr = pl.ds(pl.multiple_of(h * DP, DP), DP)

            def mx_body(kb, mx):
                ks = pl.ds(pl.multiple_of(kb * SB, SB), SB)
                st = jnp.dot(k_s[ks, grp], qm, preferred_element_type=F32)
                return jnp.maximum(mx, jnp.max(st, axis=0, keepdims=True))
            mx = jax.lax.fori_loop(0, S // SB, mx_body, jnp.full((1, NQ), -jnp.inf, F32))

            def pv_body(kb, acc):
                ks = pl.ds(pl.multiple_of(kb * SB, SB), SB)
                st = jnp.dot(k_s[ks, grp], qm, preferred_element_type=F32)
                p = jnp.exp2(st - mx).astype(BF16)
                return acc + jnp.dot(vt_s[hr, ks], p, preferred_element_type=F32)
            finish(h, jax.lax.fori_loop(0, S // SB, pv_body, jnp.zeros((DP, NQ), F32)))
            return c
        jax.lax.fori_loop(0, 2 * H, head_safe, 0)

    g = g_s[:, qcols]
    a = jnp.dot(wo_s[:, 0:512], ot_s[0:512, :], preferred_element_type=F32)
    b = jnp.dot(wo_s[:, 512:1024], ot_s[512:1024, :], preferred_element_type=F32)
    o_ref[...] = (g * a + (1.0 - g) * b).astype(o_ref.dtype)


@jax.jit
def pallas_gated_mix__mha_block__mha_block__prompt_kernel(A_x, A_wqkv, A_wo, B_x, B_wqkv, B_wo, gate_w):
    del B_x
    full = lambda a: pl.BlockSpec(a.shape, lambda i: (0,) * a.ndim)
    xt = jnp.swapaxes(A_x, 1, 2)
    args = (xt, A_wqkv, A_wo, B_wqkv, B_wo, gate_w)
    out = pl.pallas_call(
        _kernel,
        grid=(S // NQ,),
        in_specs=[pl.BlockSpec((None, D, S), lambda i: (0, 0, 0))] + [full(a) for a in args[1:]],
        out_specs=pl.BlockSpec((None, D, NQ), lambda i: (0, 0, i)),
        out_shape=jax.ShapeDtypeStruct((1, D, S), A_x.dtype),
        scratch_shapes=[pltpu.VMEM((8, 128, S), BF16), pltpu.VMEM((S, 1024), BF16), pltpu.VMEM((1024, S), BF16),
                        pltpu.VMEM((1024, NQ), BF16), pltpu.VMEM((WR, D), BF16), pltpu.VMEM((D, 1024), BF16),
                        pltpu.VMEM((1, S), F32)],
        compiler_params=pltpu.CompilerParams(dimension_semantics=("arbitrary",), vmem_limit_bytes=100 * 1024 * 1024),
    )(*args)
    return jnp.swapaxes(out, 1, 2)
```

```python
import jax
import jax.numpy as jnp
from jax.experimental import pallas as pl
from jax.experimental.pallas import tpu as pltpu

S, D, H, DH, DP = 2048, 448, 16, 28, 32
G = 4 * DH
NQ = 2048
KB = 1024
OT = 256
PT = 512
LOG2E = 1.4426950408889634
QSCALE = DH ** -0.5 * LOG2E
F32, BF16 = jnp.float32, jnp.bfloat16
HI, LO = 2.0 ** 60, 2.0 ** -60
WR = 3 * D + 16


def _tr(a):
    a = jnp.concatenate([a.astype(F32), jnp.zeros((512 - D, a.shape[1]), F32)], axis=0)
    return a.T[:, :D]


def _kernel(xt_hbm, wqa_hbm, woa_hbm, wqb_hbm, wob_hbm, gw_hbm, o_hbm,
            x_s, wq_s, wor_s, gw_s, q_s, k_s, vt_s, ot_s, w_s, wo_s, g_s, ob_s, vb_s, sem, osem):
    cp = pltpu.make_async_copy
    c_gw = cp(gw_hbm, gw_s, sem.at[0])
    c_wq = [cp(w, wq_s.at[m], sem.at[1 + m]) for m, w in enumerate((wqa_hbm, wqb_hbm))]
    c_wo = [cp(w, wor_s.at[m], sem.at[3 + m]) for m, w in enumerate((woa_hbm, wob_hbm))]
    c_x = [cp(xt_hbm.at[0, :, r * PT:(r + 1) * PT], x_s.at[:, r * PT:(r + 1) * PT], sem.at[5 + r])
           for r in range(S // PT)]
    c_wa = [cp(wqa_hbm.at[:, lo:hi], wq_s.at[0, :, lo:hi], sem.at[5 + S // PT + n])
            for n, (lo, hi) in enumerate(((0, 512), (512, 1024), (1024, 3 * D)))]
    for c in (c_wa[0], c_x[0], c_wa[1], c_wa[2], c_gw, c_x[1], c_wq[1], c_x[2], c_x[3], c_wo[0], c_wo[1]):
        c.start()

    def prep_wq(m, blocks):
        for c in blocks:
            if c + 128 <= 3 * D:
                w_s[m, c:c + 128, :] = _tr(wq_s[m, :, c:c + 128]).astype(BF16)
            else:
                w_s[m, c:3 * D, :] = _tr(wq_s[m, :, 3 * D - 128:3 * D])[c - 3 * D:, :].astype(BF16)

    def prep_wo(m):
        wop = jnp.concatenate([wor_s[m].astype(F32), jnp.zeros((D, 512 - D), F32)], axis=1)
        wop = jnp.concatenate([wop, jnp.zeros((512 - D, 512), F32)], axis=0)
        wot = wop.T[:D, :]
        if m == 0:
            wo_s[:, 0:512] = wot.astype(BF16)
        else:
            wo_s[:, 384:2 * D] = jnp.concatenate([wo_s[:, 384:D].astype(F32), wot[:, :D]], axis=1).astype(BF16)

    def proj(m, r, t=None):
        cols = slice(r * PT, (r + 1) * PT)
        nr = WR if m == 0 else 3 * D
        if t is None:
            t = jnp.dot(w_s[m, 0:nr, :], x_s[:, cols], preferred_element_type=F32)
        ri = jax.lax.broadcasted_iota(jnp.int32, (DP, PT), 0)
        tail = jnp.where(ri == DH, 1.0, 0.0)
        for j in range(4):
            q_s[m * 4 + j, 0:G, cols] = (t[j * G:(j + 1) * G, :] * QSCALE).astype(BF16)
            lo = D + j * G
            k_s[cols, (m * 4 + j) * 128:(m * 4 + j + 1) * 128] = t[lo:lo + 128, :].T.astype(BF16)
        for h in range(H):
            v = t[2 * D + h * DH:2 * D + h * DH + DP, :] if h < H - 1 else jnp.concatenate(
                [t[2 * D + h * DH:3 * D, :], jnp.zeros((DP - DH, PT), F32)], axis=0)
            vt_s[(m * H + h) * DP:(m * H + h + 1) * DP, cols] = jnp.where(ri < DH, v, tail).astype(BF16)
        vv = jnp.abs(t[2 * D:3 * D, :]).reshape(D // 8, 8, PT)
        vb_s[m, :, cols] = jnp.where(jnp.max(vv, axis=0) <= HI, 0.0, 1.0)
        if m == 0:
            g = jax.nn.sigmoid(t[3 * D:3 * D + 1, :])
            g_s[0, :, cols] = g
            g_s[1, :, cols] = 1.0 - g

    blocks = list(range(0, 3 * D, 128))
    def pdot(lo, hi, r):
        return jnp.dot(w_s[0, lo:hi, :], x_s[:, r * PT:(r + 1) * PT], preferred_element_type=F32)

    q_s[:, G:, :] = jnp.zeros((8, 128 - G, S), BF16)
    c_wa[0].wait()
    c_x[0].wait()
    prep_wq(0, blocks[0:4])
    t00 = pdot(0, 512, 0)
    for c in (c_wa[1], c_wa[2], c_gw, c_x[1]):
        c.wait()
    t10 = pdot(0, 512, 1)
    prep_wq(0, blocks[4:])
    w_s[0, 3 * D:WR, :] = jnp.broadcast_to(gw_s[...].reshape(1, D), (WR - 3 * D, D))
    proj(0, 0, jnp.concatenate([t00, pdot(512, WR, 0)], axis=0))
    proj(0, 1, jnp.concatenate([t10, pdot(512, WR, 1)], axis=0))
    for c in (c_x[2], c_x[3], c_wq[1], c_wo[0], c_wo[1]):
        c.wait()
    proj(0, 2)
    prep_wq(1, blocks[0:6])
    proj(0, 3)
    prep_wq(1, blocks[6:])
    for r in range(S // PT):
        proj(1, r)
        if r < 2:
            prep_wo(r)

    def qblock(i, carry):
        qcols = slice(0, NQ)

        def qmasked(h):
            grp = pl.ds(pl.multiple_of((h // 4) * 128, 128), 128)
            qg = q_s[h // 4, :, qcols]
            row = jax.lax.broadcasted_iota(jnp.int32, qg.shape, 0) - (h % 4) * DH
            return grp, jnp.where((row >= 0) & (row < DH), qg, jnp.zeros_like(qg))

        def norm(h, acc):
            return (acc * (g_s[h // H] / acc[DH:DH + 1, :]))[:DH, :]

        def put(j, o0, o1):
            ot_s[pl.ds(pl.multiple_of(j * 2 * DH, 8), 2 * DH), :] = jnp.concatenate([o0, o1], axis=0)

        def head(h, bad):
            grp, qm = qmasked(h)
            hr = pl.ds(pl.multiple_of(h * DP, DP), DP)
            acc = jnp.zeros((DP, NQ), F32)
            for kb in range(S // KB):
                ks = slice(kb * KB, (kb + 1) * KB)
                st = jnp.dot(k_s[ks, grp], qm, preferred_element_type=F32)
                p = jnp.exp2(st).astype(BF16)
                acc = acc + jnp.dot(vt_s[hr, ks], p, preferred_element_type=F32)
            l = acc[DH:DH + 1, :]
            return norm(h, acc), jnp.where((l >= LO) & (l <= HI), bad, 1.0)

        def pair(j, bad):
            o1, bad = head(2 * j + 1, bad)
            o0, bad = head(2 * j, bad)
            put(j, o0, o1)
            return bad
        bad = jax.lax.fori_loop(0, H, pair, jnp.zeros((1, NQ), F32))

        @pl.when(jnp.maximum(jnp.max(bad), jnp.max(vb_s[...])) > 0.0)
        def _():
            SB = 256

            def head_safe(h):
                grp, qm = qmasked(h)
                hr = pl.ds(pl.multiple_of(h * DP, DP), DP)

                def mx_body(kb, mx):
                    ks = pl.ds(pl.multiple_of(kb * SB, SB), SB)
                    st = jnp.dot(k_s[ks, grp], qm, preferred_element_type=F32)
                    return jnp.maximum(mx, jnp.max(st, axis=0, keepdims=True))
                mx = jax.lax.fori_loop(0, S // SB, mx_body, jnp.full((1, NQ), -jnp.inf, F32))

                def pv_body(kb, acc):
                    ks = pl.ds(pl.multiple_of(kb * SB, SB), SB)
                    st = jnp.dot(k_s[ks, grp], qm, preferred_element_type=F32)
                    p = jnp.exp2(st - mx).astype(BF16)
                    return acc + jnp.dot(vt_s[hr, ks], p, preferred_element_type=F32)
                return norm(h, jax.lax.fori_loop(0, S // SB, pv_body, jnp.zeros((DP, NQ), F32)))

            def pair_safe(j, c):
                put(j, head_safe(2 * j), head_safe(2 * j + 1))
                return c
            jax.lax.fori_loop(0, H, pair_safe, 0)

        outs = []
        for r in range(S // OT):
            cols = slice(r * OT, (r + 1) * OT)
            o = jnp.dot(wo_s[...], ot_s[:, cols].astype(BF16), preferred_element_type=F32)
            ob_s[:, cols] = o.astype(BF16)
            outs.append(cp(ob_s.at[:, cols], o_hbm.at[0, :, cols], osem.at[r]))
            outs[-1].start()
        for c in outs:
            c.wait()
    qblock(0, 0)


@jax.jit
def pallas_gated_mix__mha_block__mha_block__prompt_kernel(A_x, A_wqkv, A_wo, B_x, B_wqkv, B_wo, gate_w):
    del B_x
    xt = jnp.swapaxes(A_x, 1, 2)
    out = pl.pallas_call(
        _kernel,
        in_specs=[pl.BlockSpec(memory_space=pltpu.HBM)] * 6,
        out_specs=pl.BlockSpec(memory_space=pltpu.HBM),
        out_shape=jax.ShapeDtypeStruct((1, D, S), A_x.dtype),
        scratch_shapes=[
            pltpu.VMEM((D, S), BF16), pltpu.VMEM((2, D, 3 * D), BF16), pltpu.VMEM((2, D, D), BF16),
            pltpu.VMEM((D,), BF16),
            pltpu.VMEM((8, 128, S), BF16), pltpu.VMEM((S, 1024), BF16), pltpu.VMEM((1024, S), BF16),
            pltpu.VMEM((2 * D, NQ), F32), pltpu.VMEM((2, WR, D), BF16), pltpu.VMEM((D, 2 * D), BF16),
            pltpu.VMEM((2, 1, S), F32), pltpu.VMEM((D, S), BF16), pltpu.VMEM((2, 8, S), F32),
            pltpu.SemaphoreType.DMA((8 + S // PT,)), pltpu.SemaphoreType.DMA((S // OT,))],
        compiler_params=pltpu.CompilerParams(vmem_limit_bytes=100 * 1024 * 1024),
    )(xt, A_wqkv, A_wo, B_wqkv, B_wo, gate_w)
    return jnp.swapaxes(out, 1, 2)
```

```python
import jax
import jax.numpy as jnp
from jax.experimental import pallas as pl
from jax.experimental.pallas import tpu as pltpu

S, D, H, DH, DP = 2048, 448, 16, 28, 32
G = 4 * DH
KB = 1024
CG = 512
PT = 512
OT = 256
WR = 3 * D + 16
LOG2E = 1.4426950408889634
QSCALE = DH ** -0.5 * LOG2E
F32, BF16 = jnp.float32, jnp.bfloat16
L_HI, L_LO, V_HI = 2.0 ** 90, 2.0 ** -90, 2.0 ** 30
WA_PIECES = ((0, 512), (512, 1024), (1024, 3 * D))


def _tr(a):
    a = jnp.concatenate([a.astype(F32), jnp.zeros((512 - D, a.shape[1]), F32)], axis=0)
    return a.T[:, :D]


def _kernel(xt_hbm, wqa_hbm, woa_hbm, wqb_hbm, wob_hbm, gw_hbm, o_hbm,
            x_s, wq_s, wor_s, gw_s, q_s, k_s, vt_s, ot_s, w_s, wo_s, g_s, ob_s, vb_s, sem, osem):
    cp = pltpu.make_async_copy
    nx = S // PT
    c_gw = cp(gw_hbm, gw_s, sem.at[0])
    c_wb = cp(wqb_hbm, wq_s.at[1], sem.at[1])
    c_wo = [cp(w, wor_s.at[m], sem.at[2 + m]) for m, w in enumerate((woa_hbm, wob_hbm))]
    c_x = [cp(xt_hbm.at[0, :, r * PT:(r + 1) * PT], x_s.at[:, r * PT:(r + 1) * PT], sem.at[4 + r])
           for r in range(nx)]
    c_wa = [cp(wqa_hbm.at[:, lo:hi], wq_s.at[0, :, lo:hi], sem.at[4 + nx + n])
            for n, (lo, hi) in enumerate(WA_PIECES)]
    for c in (c_wa[0], c_x[0], c_wa[1], c_wa[2], c_gw, c_x[1], c_wb, c_x[2], c_x[3], c_wo[0], c_wo[1]):
        c.start()

    def prep_wq(m, blocks):
        for c in blocks:
            if c + 128 <= 3 * D:
                w_s[m, c:c + 128, :] = _tr(wq_s[m, :, c:c + 128]).astype(BF16)
            else:
                w_s[m, c:3 * D, :] = _tr(wq_s[m, :, 3 * D - 128:3 * D])[c - 3 * D:, :].astype(BF16)

    def prep_wo(m):
        wop = jnp.concatenate([wor_s[m].astype(F32), jnp.zeros((D, 512 - D), F32)], axis=1)
        wop = jnp.concatenate([wop, jnp.zeros((512 - D, 512), F32)], axis=0)
        wot = wop.T[:D, :]
        if m == 0:
            wo_s[:, 0:512] = wot.astype(BF16)
        else:
            wo_s[:, 384:2 * D] = jnp.concatenate([wo_s[:, 384:D].astype(F32), wot[:, :D]], axis=1).astype(BF16)

    def pdot(m, lo, hi, r):
        return jnp.dot(w_s[m, lo:hi, :], x_s[:, r * PT:(r + 1) * PT], preferred_element_type=F32)

    def proj(m, r, t=None):
        cols = slice(r * PT, (r + 1) * PT)
        if t is None:
            t = pdot(m, 0, WR if m == 0 else 3 * D, r)
        for j in range(4):
            q_s[m * 4 + j, 0:G, cols] = (t[j * G:(j + 1) * G, :] * QSCALE).astype(BF16)
            lo = D + j * G
            k_s[cols, (m * 4 + j) * 128:(m * 4 + j + 1) * 128] = t[lo:lo + 128, :].T.astype(BF16)
        ri = jax.lax.broadcasted_iota(jnp.int32, (DP, PT), 0)
        tail = jnp.where(ri == DH, 1.0, 0.0)
        for h in range(H):
            lo = 2 * D + h * DH
            v = t[lo:lo + DP, :] if h < H - 1 else jnp.concatenate(
                [t[lo:3 * D, :], jnp.zeros((DP - DH, PT), F32)], axis=0)
            vt_s[(m * H + h) * DP:(m * H + h + 1) * DP, cols] = jnp.where(ri < DH, v, tail).astype(BF16)
        vv = jnp.abs(t[2 * D:3 * D, :]).reshape(D // 8, 8, PT)
        vb_s[m, :, cols] = jnp.where(jnp.max(vv, axis=0) <= V_HI, 0.0, 1.0)
        if m == 0:
            g = jax.nn.sigmoid(t[3 * D:3 * D + 1, :])
            g_s[0, :, cols] = g
            g_s[1, :, cols] = 1.0 - g

    blocks = list(range(0, 3 * D, 128))
    q_s[:, G:, :] = jnp.zeros((8, 128 - G, S), BF16)
    c_wa[0].wait()
    c_x[0].wait()
    prep_wq(0, blocks[0:4])
    t00 = pdot(0, 0, 512, 0)
    for c in (c_wa[1], c_wa[2], c_gw, c_x[1]):
        c.wait()
    t10 = pdot(0, 0, 512, 1)
    prep_wq(0, blocks[4:])
    w_s[0, 3 * D:WR, :] = jnp.broadcast_to(gw_s[...].reshape(1, D), (WR - 3 * D, D))
    proj(0, 0, jnp.concatenate([t00, pdot(0, 512, WR, 0)], axis=0))
    proj(0, 1, jnp.concatenate([t10, pdot(0, 512, WR, 1)], axis=0))
    for c in (c_x[2], c_x[3], c_wb, c_wo[0], c_wo[1]):
        c.wait()
    proj(0, 2)
    prep_wq(1, blocks[0:6])
    proj(0, 3)
    prep_wq(1, blocks[6:])
    for r in range(nx):
        proj(1, r)
        if r < 2:
            prep_wo(r)

    def qmasked(h):
        grp = pl.ds(pl.multiple_of((h // 4) * 128, 128), 128)
        qg = q_s[h // 4]
        row = jax.lax.broadcasted_iota(jnp.int32, qg.shape, 0) - (h % 4) * DH
        return grp, jnp.where((row >= 0) & (row < DH), qg, jnp.zeros_like(qg))

    def norm(h, acc, cols=slice(0, S)):
        return (acc * (g_s[h // H, :, cols] / acc[DH:DH + 1, :]))[:DH, :]

    def put(j, o0, o1, cols=slice(0, S)):
        ot_s[pl.ds(pl.multiple_of(j * 2 * DH, 8), 2 * DH), cols] = jnp.concatenate([o0, o1], axis=0)

    def in_range(acc, bad):
        l = acc[DH:DH + 1, :]
        return jnp.where((l >= L_LO) & (l <= L_HI), bad, 1.0)

    def head(h, bad, sink=None):
        grp, qm = qmasked(h)
        hr = pl.ds(pl.multiple_of(h * DP, DP), DP)
        acc = jnp.zeros((DP, S), F32)
        for kb in range(S // KB):
            ks = slice(kb * KB, (kb + 1) * KB)
            st = jnp.dot(k_s[ks, grp], qm, preferred_element_type=F32)
            p = jnp.exp2(st).astype(BF16)
            if sink is not None and kb == S // KB - 1:
                bads = []
                for c in range(S // CG):
                    cols = slice(c * CG, (c + 1) * CG)
                    a = acc[:, cols] + jnp.dot(vt_s[hr, ks], p[:, cols], preferred_element_type=F32)
                    sink(norm(h, a, cols), cols)
                    bads.append(in_range(a, bad[:, cols]))
                return jnp.concatenate(bads, axis=1)
            acc = acc + jnp.dot(vt_s[hr, ks], p, preferred_element_type=F32)
        return norm(h, acc), in_range(acc, bad)

    def pair(j, bad):
        o1, bad = head(2 * j + 1, bad)
        return head(2 * j, bad, lambda o0, cols: put(j, o0, o1[:, cols], cols))

    bad = jax.lax.fori_loop(0, H, pair, jnp.zeros((1, S), F32))

    @pl.when(jnp.maximum(jnp.max(bad), jnp.max(vb_s[...])) > 0.0)
    def _():
        sb = 256

        def head_safe(h):
            grp, qm = qmasked(h)
            hr = pl.ds(pl.multiple_of(h * DP, DP), DP)

            def scores(kb):
                return jnp.dot(k_s[pl.ds(pl.multiple_of(kb * sb, sb), sb), grp], qm, preferred_element_type=F32)

            mx = jax.lax.fori_loop(
                0, S // sb, lambda kb, mx: jnp.maximum(mx, jnp.max(scores(kb), axis=0, keepdims=True)),
                jnp.full((1, S), -jnp.inf, F32))

            def pv_body(kb, acc):
                p = jnp.exp2(scores(kb) - mx).astype(BF16)
                return acc + jnp.dot(vt_s[hr, pl.ds(pl.multiple_of(kb * sb, sb), sb)], p,
                                     preferred_element_type=F32)

            return norm(h, jax.lax.fori_loop(0, S // sb, pv_body, jnp.zeros((DP, S), F32)))

        def pair_safe(j, c):
            put(j, head_safe(2 * j), head_safe(2 * j + 1))
            return c

        jax.lax.fori_loop(0, H, pair_safe, 0)

    outs = []
    for r in range(S // OT):
        cols = slice(r * OT, (r + 1) * OT)
        o = jnp.dot(wo_s[...], ot_s[:, cols].astype(BF16), preferred_element_type=F32)
        ob_s[:, cols] = o.astype(BF16)
        outs.append(cp(ob_s.at[:, cols], o_hbm.at[0, :, cols], osem.at[r]))
        outs[-1].start()
    for c in outs:
        c.wait()


@jax.jit
def pallas_gated_mix__mha_block__mha_block__prompt_kernel(A_x, A_wqkv, A_wo, B_x, B_wqkv, B_wo, gate_w):
    del B_x
    xt = jnp.swapaxes(A_x, 1, 2)
    out = pl.pallas_call(
        _kernel,
        in_specs=[pl.BlockSpec(memory_space=pltpu.HBM)] * 6,
        out_specs=pl.BlockSpec(memory_space=pltpu.HBM),
        out_shape=jax.ShapeDtypeStruct((1, D, S), A_x.dtype),
        scratch_shapes=[
            pltpu.VMEM((D, S), BF16),
            pltpu.VMEM((2, D, 3 * D), BF16),
            pltpu.VMEM((2, D, D), BF16),
            pltpu.VMEM((D,), BF16),
            pltpu.VMEM((8, 128, S), BF16),
            pltpu.VMEM((S, 1024), BF16),
            pltpu.VMEM((2 * H * DP, S), BF16),
            pltpu.VMEM((2 * D, S), F32),
            pltpu.VMEM((2, WR, D), BF16),
            pltpu.VMEM((D, 2 * D), BF16),
            pltpu.VMEM((2, 1, S), F32),
            pltpu.VMEM((D, S), BF16),
            pltpu.VMEM((2, 8, S), F32),
            pltpu.SemaphoreType.DMA((4 + S // PT + len(WA_PIECES),)),
            pltpu.SemaphoreType.DMA((S // OT,))],
        compiler_params=pltpu.CompilerParams(vmem_limit_bytes=100 * 1024 * 1024),
    )(xt, A_wqkv, A_wo, B_wqkv, B_wo, gate_w)
    return jnp.swapaxes(out, 1, 2)
```

```python
import jax
import jax.numpy as jnp
from jax.experimental import pallas as pl
from jax.experimental.pallas import tpu as pltpu

S, D, H, DH, DP = 2048, 448, 16, 28, 32
G = 4 * DH
KB = 1024
CG = 512
PT = 512
OT = 256
WR = 3 * D + 16
LOG2E = 1.4426950408889634
QSCALE = DH ** -0.5 * LOG2E
F32, BF16 = jnp.float32, jnp.bfloat16
L_HI, L_LO, V_HI = 2.0 ** 90, 2.0 ** -90, 2.0 ** 30
WA_PIECES = ((0, 256), (256, 768), (768, 3 * D))


def _tr(a):
    a = jnp.concatenate([a.astype(F32), jnp.zeros((512 - D, a.shape[1]), F32)], axis=0)
    return a.T[:, :D]


def _kernel(xt_hbm, wqa_hbm, woa_hbm, wqb_hbm, wob_hbm, gw_hbm, o_hbm,
            x_s, wq_s, wor_s, gw_s, q_s, k_s, vt_s, ot_s, w_s, wo_s, g_s, ob_s, vb_s, sem, osem):
    cp = pltpu.make_async_copy
    nx = S // PT
    c_gw = cp(gw_hbm, gw_s, sem.at[0])
    c_wb = cp(wqb_hbm, wq_s.at[1], sem.at[1])
    c_wo = [cp(w, wor_s.at[m], sem.at[2 + m]) for m, w in enumerate((woa_hbm, wob_hbm))]
    c_x = [cp(xt_hbm.at[0, :, r * PT:(r + 1) * PT], x_s.at[:, r * PT:(r + 1) * PT], sem.at[4 + r])
           for r in range(nx)]
    c_wa = [cp(wqa_hbm.at[:, lo:hi], wq_s.at[0, :, lo:hi], sem.at[4 + nx + n])
            for n, (lo, hi) in enumerate(WA_PIECES)]
    for c in (c_x[0], c_wa[0], c_wa[1], c_wa[2], c_gw, c_x[1], c_wb, c_x[2], c_x[3], c_wo[0], c_wo[1]):
        c.start()

    def prep_wq(m, blocks):
        for c in blocks:
            if c + 128 <= 3 * D:
                w_s[m, c:c + 128, :] = _tr(wq_s[m, :, c:c + 128]).astype(BF16)
            else:
                w_s[m, c:3 * D, :] = _tr(wq_s[m, :, 3 * D - 128:3 * D])[c - 3 * D:, :].astype(BF16)

    def prep_wo(m):
        wop = jnp.concatenate([wor_s[m].astype(F32), jnp.zeros((D, 512 - D), F32)], axis=1)
        wop = jnp.concatenate([wop, jnp.zeros((512 - D, 512), F32)], axis=0)
        wot = wop.T[:D, :]
        if m == 0:
            wo_s[:, 0:512] = wot.astype(BF16)
        else:
            wo_s[:, 384:2 * D] = jnp.concatenate([wo_s[:, 384:D].astype(F32), wot[:, :D]], axis=1).astype(BF16)

    def pdot(m, lo, hi, r):
        return jnp.dot(w_s[m, lo:hi, :], x_s[:, r * PT:(r + 1) * PT], preferred_element_type=F32)

    def proj(m, r, t=None):
        cols = slice(r * PT, (r + 1) * PT)
        if t is None:
            t = pdot(m, 0, WR if m == 0 else 3 * D, r)
        for j in range(4):
            q_s[m * 4 + j, 0:G, cols] = (t[j * G:(j + 1) * G, :] * QSCALE).astype(BF16)
            lo = D + j * G
            k_s[cols, (m * 4 + j) * 128:(m * 4 + j + 1) * 128] = t[lo:lo + 128, :].T.astype(BF16)
        ri = jax.lax.broadcasted_iota(jnp.int32, (DP, PT), 0)
        tail = jnp.where(ri == DH, 1.0, 0.0)
        for h in range(H):
            lo = 2 * D + h * DH
            v = t[lo:lo + DP, :] if h < H - 1 else jnp.concatenate(
                [t[lo:3 * D, :], jnp.zeros((DP - DH, PT), F32)], axis=0)
            vt_s[(m * H + h) * DP:(m * H + h + 1) * DP, cols] = jnp.where(ri < DH, v, tail).astype(BF16)
        vv = jnp.abs(t[2 * D:3 * D, :]).reshape(D // 8, 8, PT)
        vb_s[m, :, cols] = jnp.where(jnp.max(vv, axis=0) <= V_HI, 0.0, 1.0)
        if m == 0:
            g = jax.nn.sigmoid(t[3 * D:3 * D + 1, :])
            g_s[0, :, cols] = g
            g_s[1, :, cols] = 1.0 - g

    blocks = list(range(0, 3 * D, 128))
    q_s[:, G:, :] = jnp.zeros((8, 128 - G, S), BF16)
    c_wa[0].wait()
    c_x[0].wait()
    prep_wq(0, blocks[0:2])
    t00 = pdot(0, 0, 256, 0)
    c_wa[1].wait()
    prep_wq(0, blocks[2:6])
    t01 = pdot(0, 256, 768, 0)
    for c in (c_wa[2], c_gw, c_x[1]):
        c.wait()
    t10 = pdot(0, 0, 768, 1)
    prep_wq(0, blocks[6:])
    w_s[0, 3 * D:WR, :] = jnp.broadcast_to(gw_s[...].reshape(1, D), (WR - 3 * D, D))
    proj(0, 0, jnp.concatenate([t00, t01, pdot(0, 768, WR, 0)], axis=0))
    proj(0, 1, jnp.concatenate([t10, pdot(0, 768, WR, 1)], axis=0))
    for c in (c_x[2], c_x[3], c_wb, c_wo[0], c_wo[1]):
        c.wait()
    proj(0, 2)
    prep_wq(1, blocks[0:6])
    proj(0, 3)
    prep_wq(1, blocks[6:])
    for r in range(nx):
        proj(1, r)
        if r < 2:
            prep_wo(r)

    def qmasked(h):
        grp = pl.ds(pl.multiple_of((h // 4) * 128, 128), 128)
        qg = q_s[h // 4]
        row = jax.lax.broadcasted_iota(jnp.int32, qg.shape, 0) - (h % 4) * DH
        return grp, jnp.where((row >= 0) & (row < DH), qg, jnp.zeros_like(qg))

    def norm(h, acc, cols=slice(0, S)):
        return (acc * (g_s[h // H, :, cols] / acc[DH:DH + 1, :]))[:DH, :]

    def put(j, o0, o1, cols=slice(0, S)):
        ot_s[pl.ds(pl.multiple_of(j * 2 * DH, 8), 2 * DH), cols] = jnp.concatenate([o0, o1], axis=0)

    def in_range(acc, bad):
        l = acc[DH:DH + 1, :]
        return jnp.where((l >= L_LO) & (l <= L_HI), bad, 1.0)

    def head(h, bad, sink=None):
        grp, qm = qmasked(h)
        hr = pl.ds(pl.multiple_of(h * DP, DP), DP)
        acc = jnp.zeros((DP, S), F32)
        for kb in range(S // KB):
            ks = slice(kb * KB, (kb + 1) * KB)
            st = jnp.dot(k_s[ks, grp], qm, preferred_element_type=F32)
            p = jnp.exp2(st).astype(BF16)
            if sink is not None and kb == S // KB - 1:
                bads = []
                for c in range(S // CG):
                    cols = slice(c * CG, (c + 1) * CG)
                    a = acc[:, cols] + jnp.dot(vt_s[hr, ks], p[:, cols], preferred_element_type=F32)
                    sink(norm(h, a, cols), cols)
                    bads.append(in_range(a, bad[:, cols]))
                return jnp.concatenate(bads, axis=1)
            acc = acc + jnp.dot(vt_s[hr, ks], p, preferred_element_type=F32)
        return norm(h, acc), in_range(acc, bad)

    def pair(j, bad):
        o1, bad = head(2 * j + 1, bad)
        return head(2 * j, bad, lambda o0, cols: put(j, o0, o1[:, cols], cols))

    bad = jax.lax.fori_loop(0, H, pair, jnp.zeros((1, S), F32))

    @pl.when(jnp.maximum(jnp.max(bad), jnp.max(vb_s[...])) > 0.0)
    def _():
        sb = 256

        def head_safe(h):
            grp, qm = qmasked(h)
            hr = pl.ds(pl.multiple_of(h * DP, DP), DP)

            def scores(kb):
                return jnp.dot(k_s[pl.ds(pl.multiple_of(kb * sb, sb), sb), grp], qm, preferred_element_type=F32)

            mx = jax.lax.fori_loop(
                0, S // sb, lambda kb, mx: jnp.maximum(mx, jnp.max(scores(kb), axis=0, keepdims=True)),
                jnp.full((1, S), -jnp.inf, F32))

            def pv_body(kb, acc):
                p = jnp.exp2(scores(kb) - mx).astype(BF16)
                return acc + jnp.dot(vt_s[hr, pl.ds(pl.multiple_of(kb * sb, sb), sb)], p,
                                     preferred_element_type=F32)

            return norm(h, jax.lax.fori_loop(0, S // sb, pv_body, jnp.zeros((DP, S), F32)))

        def pair_safe(j, c):
            put(j, head_safe(2 * j), head_safe(2 * j + 1))
            return c

        jax.lax.fori_loop(0, H, pair_safe, 0)

    outs = []
    for r in range(S // OT):
        cols = slice(r * OT, (r + 1) * OT)
        o = jnp.dot(wo_s[...], ot_s[:, cols].astype(BF16), preferred_element_type=F32)
        ob_s[:, cols] = o.astype(BF16)
        outs.append(cp(ob_s.at[:, cols], o_hbm.at[0, :, cols], osem.at[r]))
        outs[-1].start()
    for c in outs:
        c.wait()


@jax.jit
def pallas_gated_mix__mha_block__mha_block__prompt_kernel(A_x, A_wqkv, A_wo, B_x, B_wqkv, B_wo, gate_w):
    del B_x
    xt = jnp.swapaxes(A_x, 1, 2)
    out = pl.pallas_call(
        _kernel,
        in_specs=[pl.BlockSpec(memory_space=pltpu.HBM)] * 6,
        out_specs=pl.BlockSpec(memory_space=pltpu.HBM),
        out_shape=jax.ShapeDtypeStruct((1, D, S), A_x.dtype),
        scratch_shapes=[
            pltpu.VMEM((D, S), BF16),
            pltpu.VMEM((2, D, 3 * D), BF16),
            pltpu.VMEM((2, D, D), BF16),
            pltpu.VMEM((D,), BF16),
            pltpu.VMEM((8, 128, S), BF16),
            pltpu.VMEM((S, 1024), BF16),
            pltpu.VMEM((2 * H * DP, S), BF16),
            pltpu.VMEM((2 * D, S), F32),
            pltpu.VMEM((2, WR, D), BF16),
            pltpu.VMEM((D, 2 * D), BF16),
            pltpu.VMEM((2, 1, S), F32),
            pltpu.VMEM((D, S), BF16),
            pltpu.VMEM((2, 8, S), F32),
            pltpu.SemaphoreType.DMA((4 + S // PT + len(WA_PIECES),)),
            pltpu.SemaphoreType.DMA((S // OT,))],
        compiler_params=pltpu.CompilerParams(vmem_limit_bytes=100 * 1024 * 1024),
    )(xt, A_wqkv, A_wo, B_wqkv, B_wo, gate_w)
    return jnp.swapaxes(out, 1, 2)
```
